```python
import os as _os
_os.environ.setdefault("JAX_PLATFORMS", "cpu")
import jax
import jax.numpy as jnp

def _softmax(x, axis=-1):
    return jax.nn.softmax(x, axis=axis)
def _gelu(x):
    return jax.nn.gelu(x, approximate=True)
def _silu(x):
    return jax.nn.silu(x)
def _sigmoid(x):
    return jax.nn.sigmoid(x)
def _layernorm(x, axis=-1, eps=1e-5):
    m = jnp.mean(x, axis=axis, keepdims=True)
    v = jnp.var(x, axis=axis, keepdims=True)
    return (x - m) / jnp.sqrt(v + eps)
def _scatter_add(tgt, idx, src, axis=0):
    return tgt.at[idx].add(src)
def _segment_sum(src, seg, n):
    return jax.ops.segment_sum(src, seg, n)
class _Rng:
    def __init__(self, key):
        self._k = key
    def _next(self):
        self._k, sub = jax.random.split(self._k)
        return sub
    def normal(self, shape):
        return jax.random.normal(self._next(), shape, dtype=jnp.bfloat16)
    def randint(self, lo, hi, shape):
        return jax.random.randint(self._next(), shape, lo, hi, dtype=jnp.int32)
    def uniform(self, shape, lo=0.0, hi=1.0):
        return jax.random.uniform(self._next(), shape, jnp.bfloat16, lo, hi)
    def permutation(self, n):
        return jax.random.permutation(self._next(), n)


kernel_name = 'gated_mix__linear_attn_block__sliding_local_dilated__prompt'

def setup_inputs():
    _rng = _Rng(jax.random.key(int.from_bytes(__import__("os").urandom(4), "little")))
    _w = (lambda a: (lambda t: t.astype(jnp.bfloat16) if jnp.issubdtype(t.dtype, jnp.floating) else t)(jnp.asarray(a)))
    def _A_setup():
        B, S, D = 1, 2048, 512
        return {
            "x": _w((lambda *s: _rng.normal(s) * 0.05)(B, S, D)),
            "wqkv": _w((lambda *s: _rng.normal(s) * 1.6)(D, 3 * D)),
            "wo": _w((lambda *s: _rng.normal(s) * 0.8)(D, D)),
        }
    _A_in = _A_setup()

    def _B_setup():
        B, S, D = 1, 2048, 512
        return {
            "x": _w((lambda *s: _rng.normal(s) * 0.05)(B, S, D)),
            "wqkv": _w((lambda *s: _rng.normal(s) * 0.8)(D, 3 * D)),
            "wo": _w((lambda *s: _rng.normal(s) * 0.05)(D, D)),
        }
    _B_in = _B_setup()

    return {
        "A_x": _A_in["x"],
        "A_wqkv": _A_in["wqkv"],
        "A_wo": _A_in["wo"],
        "B_x": _B_in["x"],
        "B_wqkv": _B_in["wqkv"],
        "B_wo": _B_in["wo"],
        "gate_w": _w((lambda *s: _rng.normal(s) * 0.05)(512) * 16.0),
    }

def reference(A_x, A_wqkv, A_wo, B_x, B_wqkv, B_wo, gate_w):
    def _A_ref(x, wqkv, wo):
        B, S, D = x.shape
        H = 32; Dh = D // H
        qkv = (lambda x, *d: x.transpose(*d))((x @ wqkv).reshape(B, S, 3, H, Dh), 2, 0, 3, 1, 4)
        q, k, v = qkv[0], qkv[1], qkv[2]
        phi = lambda t: jnp.where(t > 0, t + 1, jnp.exp(t)) + 1e-6
        pq, pk = phi(q), phi(k)
        kv = jnp.einsum("bhsd,bhse->bhde", pk, v)
        z = jnp.einsum("bhsd->bhd", pk)
        num = jnp.einsum("bhqd,bhde->bhqe", pq, kv)
        den = jnp.einsum("bhqd,bhd->bhq", pq, z)[..., None] + 1e-6
        o = num / den
        return (lambda x, *d: x.transpose(*d))(o, 0, 2, 1, 3).reshape(B, S, D) @ wo

    def _B_ref(x, wqkv, wo):
        B, S, D = x.shape
        H = 32; Dh = D // H
        W, dil = 8, 2
        qkv = (lambda x, *d: x.transpose(*d))((x @ wqkv).reshape(B, S, 3, H, Dh), 2, 0, 3, 1, 4)
        q, k, v = qkv[0], qkv[1], qkv[2]
        scale = Dh ** -0.5
        pos = jnp.arange(S)
        off = jnp.arange(W) * dil
        idx = pos[:, None] - off[None, :]
        mask = idx >= 0
        idx_c = jnp.where(mask, idx, 0).reshape(-1)
        kg = k[:, :, idx_c, :].reshape(B, H, S, W, Dh)
        vg = v[:, :, idx_c, :].reshape(B, H, S, W, Dh)
        logits = jnp.einsum("bhsd,bhswd->bhsw", q, kg) * scale
        logits = jnp.where(mask[None, None, :, :], logits, -1e9)
        attn = _softmax(logits, axis=-1)
        o = jnp.einsum("bhsw,bhswd->bhsd", attn, vg)
        return (lambda x, *d: x.transpose(*d))(o, 0, 2, 1, 3).reshape(B, S, D) @ wo

    x = A_x
    g = _sigmoid((x * gate_w).sum(-1, keepdims=True))
    a = _A_ref(x, A_wqkv, A_wo)
    b = _B_ref(x, B_wqkv, B_wo)
    return g * a + (1 - g) * b
```

```python
import jax
import jax.numpy as jnp
from jax import lax
import jax.experimental.pallas as pl
import jax.experimental.pallas.tpu as pltpu

S, D = 2048, 512
T = 512
ST = 256
MR = 128
R = 16
NT, NS = S // T, S // ST
BF, F32 = jnp.bfloat16, jnp.float32
HALO = 16
WR = D // NT


def _dot(a, b):
    return jnp.dot(a, b, preferred_element_type=F32)


def _phi(t):
    return jnp.where(t > 0, t + 1.0, jnp.exp(t)) + 1e-6


def _perm_cols(w):
    wi = pltpu.bitcast(w, jnp.int32)
    lane = lax.broadcasted_iota(jnp.int32, (wi.shape[0], 128), 1)
    outs = []
    for t in range(4):
        idx = (lane % 8) * 16 + 4 * t + lane // 32
        o = None
        for u in range(4):
            g = jnp.take_along_axis(wi[:, 128 * u:128 * (u + 1)], idx, axis=1)
            o = g if o is None else jnp.where((lane % 32) // 8 == u, g, o)
        outs.append(pltpu.bitcast(o, BF))
    return outs


def _merge(a, b):
    ia = ib = 0
    while ia < len(a) or ib < len(b):
        if ib >= len(b) or (ia < len(a) and ia * len(b) <= ib * len(a)):
            a[ia]()
            ia += 1
        else:
            b[ib]()
            ib += 1


def _kernel(x_hbm, aw_hbm, awo_hbm, bw_hbm, bwo_hbm, gw_ref, o_hbm,
            x_ref, aw_ref, awo_ref, bw_ref, bwo_ref, bwp_ref, wof_ref, m_ref,
            kv_ref, z_ref, zb_ref, g_ref, q_ref, kb_ref, vb_ref, u_ref, o_ref,
            sx, sw, sb, so):
    def pk_(a):
        return pltpu.bitcast(a, jnp.int32)

    def hv(rows):
        return pl.ds(pl.multiple_of(rows.start // 2, rows.size // 2), rows.size // 2)

    def lt(n):
        return slice(128 * n, 128 * (n + 1))

    def x_cp(i, g):
        rows = pl.ds(i * T, T)
        return pltpu.make_async_copy(x_hbm.at[rows, :], x_ref.at[rows, :], sx.at[i, g])

    def aw_cp(n):
        return pltpu.make_async_copy(aw_hbm.at[:, D * n:D * (n + 1)], aw_ref.at[n], sw.at[n])

    def x0_cp(c):
        rows = pl.ds(c * 128, 128)
        return pltpu.make_async_copy(x_hbm.at[rows, :], x_ref.at[rows, :], sx.at[0, c])

    def wk_cp(c):
        return pltpu.make_async_copy(aw_hbm.at[:, D + 128 * c:D + 128 * (c + 1)], aw_ref.at[1, :, lt(c)], sw.at[4 + c])

    def bw_cp(i):
        rows = pl.ds(i * WR, WR)
        return pltpu.make_async_copy(bw_hbm.at[rows, :], bw_ref.at[rows, :], sb.at[i])

    awo_cp = pltpu.make_async_copy(awo_hbm, awo_ref, sw.at[12])
    bwo_cp = pltpu.make_async_copy(bwo_hbm, bwo_ref, sw.at[13])

    def o_cp(s):
        rows = pl.ds(s * ST, ST)
        return pltpu.make_async_copy(o_ref.at[rows, :], o_hbm.at[rows, :], so.at[s])

    for c in range(4):
        x0_cp(c).start()
        wk_cp(c).start()
    x_cp(1, 0).start()
    aw_cp(0).start()
    bwo_cp.start()
    bw_cp(0).start()
    bw_cp(1).start()
    x_cp(2, 0).start()
    bw_cp(2).start()
    x_cp(3, 0).start()
    bw_cp(3).start()
    aw_cp(2).start()
    awo_cp.start()

    r = lax.broadcasted_iota(jnp.int32, (128, 128), 0)
    c = lax.broadcasted_iota(jnp.int32, (128, 128), 1)
    bd = (r // 16) == (c // 16)

    kv_ref[...] = jnp.zeros_like(kv_ref)
    z_ref[...] = jnp.zeros_like(z_ref)
    kb_ref[:, 0:HALO, :] = jnp.zeros((4, HALO, 128), F32)
    vb_ref[:, 0:HALO, :] = jnp.zeros((4, HALO, 128), F32)
    def load_x(rows):
        return x_ref[rows, :]

    gw = gw_ref[...].astype(F32).reshape(1, D)

    def gate_k(rows, n):
        x = load_x(rows)
        gate = jax.nn.sigmoid(jnp.sum(x.astype(F32) * gw, axis=-1, keepdims=True))
        g_ref[rows, :] = jnp.broadcast_to(gate, (n, 128))
        return x

    def acc_kv(x, pka):
        z_ref[...] += jnp.sum(pka, axis=0, keepdims=True)
        kv_ref[...] += lax.dot_general(x, pka.astype(BF), (((0,), (0,)), ((), ())), preferred_element_type=F32)

    for c in range(4):
        wk_cp(c).wait()
        x0_cp(c).wait()
    x = gate_k(pl.ds(0, T), T)
    acc_kv(x, _phi(_dot(x, aw_ref[1])))

    aw_cp(0).wait()
    bwo_cp.wait()
    bw_cp(0).wait()
    for g in range(4):
        wof_ref[g] = bwo_ref[:, lt(g)].astype(F32)
    for ds in range(4):
        for g in range(4):
            m_ref[g, hv(pl.ds(D + 32 * ds, 32)), :] = pk_(wof_ref[g, pl.ds(ds, 32, stride=16), :].astype(BF))

    PR = 192

    def phase1(i, carry):
        x_cp(i, 0).wait()
        bw_cp(i).wait()
        rows = pl.ds(pl.multiple_of(i * T, T), T)
        wrows = pl.ds(pl.multiple_of(jnp.minimum((i - 1) * PR, D - PR), 64), PR)
        x = gate_k(rows, T)
        acc_kv(x, _phi(_dot(x, aw_ref[1])))
        for g in range(4):
            if g == 3:
                outs = _perm_cols(aw_ref[0, wrows, :])
                for t in range(4):
                    bwp_ref[12 + t, hw(wrows), :] = pk_(outs[t])
            if g < 3:
                outs = _perm_cols(bw_ref[wrows, D * g:D * (g + 1)])
                for t in range(4):
                    bwp_ref[4 * g + t, hw(wrows), :] = pk_((outs[t].astype(F32) * 0.25).astype(BF) if g == 0 else outs[t])
        for ds in range(4):
            for g in range(4):
                m_ref[g, hv(pl.ds(D + 128 * i + 32 * ds, 32)), :] = pk_(wof_ref[g, pl.ds(4 * i + ds, 32, stride=16), :].astype(BF))
        return carry

    def hw(rows):
        return pl.ds(pl.multiple_of(rows.start // 2, 32), rows.size // 2)

    lax.fori_loop(1, NT, phase1, 0)

    for n in (2,):
        aw_cp(n).wait()
    awo_cp.wait()
    z = z_ref[...]
    for g in range(4):
        kvg = lax.dot_general(kv_ref[:, lt(g)].astype(BF), aw_ref[2, :, lt(g)], (((0,), (0,)), ((), ())), preferred_element_type=F32)
        kvg = jnp.where(bd, kvg, 0.0).astype(BF)
        mg = _dot(kvg, awo_ref[lt(g), :])
        for n in range(4):
            wof_ref[n, lt(g), :] = mg[:, lt(n)]
    for t in range(4):
        for ds in range(4):
            for n in range(4):
                m_ref[n, hv(pl.ds(128 * t + 32 * ds, 32)), :] = pk_(wof_ref[n, pl.ds(4 * t + ds, 32, stride=16), :].astype(BF))
    zb = jnp.broadcast_to(z, (8, D))
    lane = lax.broadcasted_iota(jnp.int32, (8, 128), 1)
    for t in range(4):
        o = None
        for u in range(4):
            gg = jnp.take_along_axis(zb[:, lt(u)], (lane % 8) * 16 + 4 * t + lane // 32, axis=1)
            o = gg if o is None else jnp.where((lane % 32) // 8 == u, gg, o)
        zb_ref[t] = o
    ones = jnp.where((r % 32) == (c % 32), 0.25, 0.0).astype(BF)

    def wcat(ref, n0):
        return jnp.concatenate([pltpu.bitcast(ref[n0 + n], BF) for n in range(4)], axis=1)

    def proj_thunks(s):
        th = []

        def a_tile(c):
            rows = pl.ds(pl.multiple_of(s * ST + c * MR, MR), MR)
            pq = _phi(_dot(load_x(rows), wcat(bwp_ref, 12)))
            den = None
            for g in range(4):
                pr = pq[:, lt(g)] * zb_ref[g, 0:1, :]
                den = pr if den is None else den + pr
            den = den + pltpu.roll(den, 64, 1)
            den = den + pltpu.roll(den, 32, 1)
            sc = g_ref[rows, :] / (den + 1e-6)
            for g in range(4):
                u_ref[g, hv(rows), :] = pk_((pq[:, lt(g)] * sc).astype(BF))

        def b_tile(c, n):
            rows = pl.ds(pl.multiple_of(s * ST + c * MR, MR), MR)
            hrows = pl.ds(pl.multiple_of(s * ST + c * MR, MR) + HALO, MR)
            y = _dot(load_x(rows), wcat(bwp_ref, 4 * n))
            for t in range(4):
                if n == 0:
                    q_ref[t, rows, :] = y[:, lt(t)]
                elif n == 1:
                    kb_ref[t, hrows, :] = y[:, lt(t)]
                else:
                    vb_ref[t, hrows, :] = y[:, lt(t)]

        for c in range(ST // MR):
            for n in range(3):
                th.append(lambda c=c, n=n: b_tile(c, n))
            th.append(lambda c=c: a_tile(c))
        return th

    def out_thunks(s):
        def o_tile(c):
            rows = pl.ds(pl.multiple_of(s * ST + c * MR, MR), MR)
            u = jnp.concatenate([pltpu.bitcast(u_ref[g, hv(rows), :], BF) for g in range(8)], axis=1)
            o_ref[rows, :] = _dot(u, wcat(m_ref, 0)).astype(BF)

        return [lambda c=c: o_tile(c) for c in range(ST // MR)]

    H = ST // 2

    def attn_thunks(s, first):
        base = pl.multiple_of(s * ST, ST)

        def ew1(hf, cc):
            r0 = H * hf + R * cc
            qs = [q_ref[t, pl.ds(base + r0, R), :] for t in range(4)]
            ls = []
            for j in range(8):
                p = None
                for t in range(4):
                    pr = qs[t] * kb_ref[t, pl.ds(base + (HALO + r0 - 2 * j), R), :]
                    p = pr if p is None else p + pr
                p = p + pltpu.roll(p, 64, 1)
                p = p + pltpu.roll(p, 32, 1)
                ls.append(p)
            ew2(hf, cc, ls)

        def red(hf):
            pass

        def ew2(hf, cc, ls):
            r0 = H * hf + R * cc
            if first and r0 == 0:
                row = lax.broadcasted_iota(jnp.int32, (R, 128), 0)
                ls = [jnp.where(row >= 2 * j, ls[j], -1e9) for j in range(8)]
            m = ls[0]
            for l in ls[1:]:
                m = jnp.maximum(m, l)
            es = [jnp.exp(l - m) for l in ls]
            den = es[0]
            for e in es[1:]:
                den = den + e
            sc = (1.0 - g_ref[pl.ds(base + r0, R), :]) / den
            for t in range(4):
                o = None
                for j in range(8):
                    tt = es[j] * vb_ref[t, pl.ds(base + (HALO + r0 - 2 * j), R), :]
                    o = tt if o is None else o + tt
                u_ref[4 + t, hv(pl.ds(base + r0, R)), :] = pk_((o * sc).astype(BF))

        n = H // R
        th = [lambda hf=hf, cc=cc: ew1(hf, cc) for hf in range(2) for cc in range(n)]
        return th

    if True:
        for f in proj_thunks(0):
            f()
        _merge(proj_thunks(1), attn_thunks(0, True))

    def tail():
        _merge(out_thunks(NS - 2), attn_thunks(NS - 1, False))
        o_cp(NS - 2).start()
        for f in out_thunks(NS - 1):
            f()
        o_cp(NS - 1).start()
        for s in range(NS):
            o_cp(s).wait()

    def phase2(s, carry):
        _merge(proj_thunks(s + 1) + out_thunks(s - 1), attn_thunks(s, False))
        o_cp(s - 1).start()
        return carry

    if True:
        for k in range(1, NS - 1):
            phase2(k, 0)
    if True:
      tail()


@jax.jit
def pallas_gated_mix__linear_attn_block__sliding_local_dilated__prompt_kernel(
    A_x, A_wqkv, A_wo, B_x, B_wqkv, B_wo, gate_w):
    del B_x
    hbm = pl.BlockSpec(memory_space=pl.ANY)
    V = pltpu.VMEM
    out = pl.pallas_call(
        _kernel,
        in_specs=[hbm, hbm, hbm, hbm, hbm, pl.BlockSpec(memory_space=pltpu.VMEM)],
        out_specs=hbm,
        out_shape=jax.ShapeDtypeStruct((S, D), BF),
        scratch_shapes=[
            V((S, D), BF), V((3, D, D), BF), V((D, D), BF), V((D, 3 * D), BF), V((D, D), BF),
            V((16, D // 2, 128), jnp.int32), V((4, D, 128), F32), V((4, D, 128), jnp.int32),
            V((D, D), F32), V((1, D), F32), V((4, 8, 128), F32), V((S, 128), F32),
            V((4, S, 128), F32), V((4, S + HALO, 128), F32), V((4, S + HALO, 128), F32),
            V((8, S // 2, 128), jnp.int32), V((S, D), BF),
            pltpu.SemaphoreType.DMA((NT, 4)), pltpu.SemaphoreType.DMA((14,)),
            pltpu.SemaphoreType.DMA((NT,)), pltpu.SemaphoreType.DMA((NS,)),
        ],
        compiler_params=pltpu.CompilerParams(vmem_limit_bytes=100 * 1024 * 1024),
    )(A_x.reshape(S, D), A_wqkv, A_wo, B_wqkv, B_wo, gate_w)
    return out.reshape(1, S, D)
```
